```python
import jax
import jax.numpy as jnp

def _softmax(x, axis=-1):
    return jax.nn.softmax(x, axis=axis)

def _gelu(x):
    return jax.nn.gelu(x, approximate=True)

def _silu(x):
    return jax.nn.silu(x)

def _sigmoid(x):
    return jax.nn.sigmoid(x)

def _layernorm(x, axis=-1, eps=1e-05):
    m = jnp.mean(x, axis=axis, keepdims=True)
    v = jnp.var(x, axis=axis, keepdims=True)
    return (x - m) / jnp.sqrt(v + eps)

def _scatter_add(tgt, idx, src, axis=0):
    return tgt.at[idx].add(src)

def _segment_sum(src, seg, n):
    return jax.ops.segment_sum(src, seg, n)

class _Rng:

    def __init__(self, key):
        self._k = key

    def _next(self):
        self._k, sub = jax.random.split(self._k)
        return sub

    def normal(self, shape):
        return jax.random.normal(self._next(), shape, dtype=jnp.bfloat16)

    def randint(self, lo, hi, shape):
        return jax.random.randint(self._next(), shape, lo, hi, dtype=jnp.int32)

    def uniform(self, shape, lo=0.0, hi=1.0):
        return jax.random.uniform(self._next(), shape, jnp.bfloat16, lo, hi)

    def permutation(self, n):
        return jax.random.permutation(self._next(), n)
kernel_name = 'adaLN_cond__sliding_block_cached__mixer_gmlp__decode'

def setup_inputs():
    _rng = _Rng(jax.random.key(int.from_bytes(__import__("os").urandom(4), "little")))
    _w = lambda a: (lambda t: t.astype(jnp.bfloat16) if jnp.issubdtype(t.dtype, jnp.floating) else t)(jnp.asarray(a))

    def _A_setup():
        B, Sq, D = (1, 1, 448)
        Hq, Hkv, Sk, Dh = (16, 8, 65536, 256)
        assert Hq % Hkv == 0, (Hq, Hkv)
        return {'x': _w((lambda *s: _rng.normal(s) * 0.05)(B, Sq, D)), 'k_cache': _w((lambda *s: _rng.normal(s) * 0.05)(B, Hkv, Sk, Dh)), 'v_cache': _w((lambda *s: _rng.normal(s) * 0.05)(B, Hkv, Sk, Dh)), 'wq': _w((lambda *s: _rng.normal(s) * 0.05)(D, Hq * Dh) * D ** (-0.5)), 'wo': _w((lambda *s: _rng.normal(s) * 0.05)(Hq * Dh, D) * (Hq * Dh) ** (-0.5))}
    _A_in = _A_setup()

    def _B_setup():
        B, S, D, F = (1, 1, 448, 1792)
        Fh = F // 2
        return {'x': _w((lambda *s: _rng.normal(s) * 0.05)(B, S, D)), 'w_in': _w((lambda *s: _rng.normal(s) * 0.05)(D, 2 * Fh)), 'w_sp': _w(0.01 * (lambda *s: _rng.normal(s) * 0.05)(S, S)), 'b_sp': _w(1.0 + 0.01 * (lambda *s: _rng.normal(s) * 0.05)(S)), 'w_out': _w((lambda *s: _rng.normal(s) * 0.05)(Fh, D))}
    _B_in = _B_setup()
    return {'A_x': _A_in['x'], 'A_k_cache': _A_in['k_cache'], 'A_v_cache': _A_in['v_cache'], 'A_wq': _A_in['wq'], 'A_wo': _A_in['wo'], 'B_x': _B_in['x'], 'B_w_in': _B_in['w_in'], 'B_w_sp': _B_in['w_sp'], 'B_b_sp': _B_in['b_sp'], 'B_w_out': _B_in['w_out'], 'c': _w((lambda *s: _rng.normal(s) * 0.05)(1, 448)), 'w_mod': _w((lambda *s: _rng.normal(s) * 0.05)(448, 6 * 448) * 448 ** (-0.5))}

def reference(A_x, A_k_cache, A_v_cache, A_wq, A_wo, B_x, B_w_in, B_w_sp, B_b_sp, B_w_out, c, w_mod):

    def _A_ref(x, k_cache, v_cache, wq, wo):
        B, Sq, D = x.shape
        Hq, Dh = (16, 256)
        Hkv, Sk = (k_cache.shape[1], k_cache.shape[2])
        W = min(4096, max(256, Sk // 4))
        rep = Hq // Hkv
        q = (lambda x, *d: x.transpose(*d))((x @ wq).reshape(B, Sq, Hq, Dh), 0, 2, 1, 3)
        k = jnp.repeat(k_cache[:, :, Sk - W:, :], rep, axis=1)
        v = jnp.repeat(v_cache[:, :, Sk - W:, :], rep, axis=1)
        scores = jnp.einsum('bhqd,bhkd->bhqk', q, k) * Dh ** (-0.5)
        p = _softmax(scores, axis=-1)
        o = jnp.einsum('bhqk,bhkd->bhqd', p, v)
        return (lambda x, *d: x.transpose(*d))(o, 0, 2, 1, 3).reshape(B, Sq, Hq * Dh) @ wo

    def _B_ref(x, w_in, w_sp, b_sp, w_out):
        B, S, D = x.shape
        F = w_in.shape[-1]
        Fh = F // 2
        z = _gelu(jnp.einsum('bsd,df->bsf', x, w_in))
        z1 = z[..., :Fh].copy()
        z2 = _layernorm(z[..., Fh:], axis=-1)
        g = jnp.einsum('ts,bsf->btf', w_sp, z2) + b_sp[None, :, None]
        return jnp.einsum('bsf,fd->bsd', z1 * g, w_out)
    x = A_x
    mod = (_silu(c) @ w_mod).reshape(c.shape[0], 6, 1, -1)
    sa, ca, ga, sb, cb, gb = (mod[:, 0].copy(), mod[:, 1].copy(), mod[:, 2].copy(), mod[:, 3].copy(), mod[:, 4].copy(), mod[:, 5].copy())
    h = _layernorm(x, axis=-1) * (1 + ca) + sa
    x = x + ga * _A_ref(h, A_k_cache, A_v_cache, A_wq, A_wo)
    h = _layernorm(x, axis=-1) * (1 + cb) + sb
    x = x + gb * _B_ref(h, B_w_in, B_w_sp, B_b_sp, B_w_out)
    return x
```

```python
import jax
import jax.numpy as jnp
from jax import lax
import jax.experimental.pallas as pl
import jax.experimental.pallas.tpu as pltpu

D = 448
HQ, HKV, DH = 16, 8, 256
FH = 896
EPS = 1e-5
BF16 = jnp.bfloat16
F32 = jnp.float32

_NT = (((1,), (1,)), ((), ()))

_OUT_CHUNKS = ((0, 128), (128, 256), (256, 384), (384, 448))


def _layernorm(x):
    m = jnp.mean(x, axis=-1, keepdims=True)
    xc = x - m
    v = jnp.mean(xc * xc, axis=-1, keepdims=True)
    return xc * lax.rsqrt(v + EPS)


def _rows8(x):
    return jnp.broadcast_to(x, (8, x.shape[-1]))


def _make_kernel(sk, w):
    n_chunks = len(_OUT_CHUNKS)
    S_C, S_X, S_MOD, S_WQ, S_WSP, S_BSP = range(6)
    S_K, S_V = 6, 6 + HKV
    S_WO, S_WIN2, S_WIN1, S_WOUT = range(6 + 2 * HKV, 10 + 2 * HKV)
    n_sems = S_WOUT + n_chunks
    X, GA, SB, CB, GB, X1 = range(6)

    def kernel(x_hbm, k_hbm, v_hbm, wq_hbm, wot_hbm, win_hbm, wsp_hbm, bsp_hbm,
               woutt_hbm, c_hbm, wmod_hbm,
               o_ref,
               x_v, c_v, wsp_v, bsp_v, wmod_v, wq_v, k_v, v_v, wot_v, win_v,
               woutt_v, q_s, o_s, vec_s):

        def body(sems):
            cp = pltpu.make_async_copy
            cp_c = cp(c_hbm, c_v, sems.at[S_C])
            cp_x = cp(x_hbm, x_v, sems.at[S_X])
            cp_mod = cp(wmod_hbm, wmod_v, sems.at[S_MOD])
            cp_wq = cp(wq_hbm, wq_v, sems.at[S_WQ])
            cp_wsp = cp(wsp_hbm, wsp_v, sems.at[S_WSP])
            cp_bsp = cp(bsp_hbm, bsp_v, sems.at[S_BSP])

            def cp_k(h):
                return cp(k_hbm.at[0, h, pl.ds(sk - w, w), :], k_v.at[h],
                          sems.at[S_K + h])

            def cp_v(h):
                return cp(v_hbm.at[0, h, pl.ds(sk - w, w), :], v_v.at[h],
                          sems.at[S_V + h])

            cp_wo = cp(wot_hbm, wot_v, sems.at[S_WO])
            cp_win2 = cp(win_hbm.at[:, pl.ds(FH, FH)], win_v.at[:, pl.ds(FH, FH)],
                         sems.at[S_WIN2])
            cp_win1 = cp(win_hbm.at[:, pl.ds(0, FH)], win_v.at[:, pl.ds(0, FH)],
                         sems.at[S_WIN1])
            cp_wout = [
                cp(woutt_hbm.at[pl.ds(r0, r1 - r0), :],
                   woutt_v.at[pl.ds(r0, r1 - r0), :], sems.at[S_WOUT + i])
                for i, (r0, r1) in enumerate(_OUT_CHUNKS)
            ]

            cp_c.start()
            cp_x.start()
            cp_mod.start()
            cp_wq.start()
            cp_wsp.start()
            cp_bsp.start()
            for h in range(HKV):
                cp_k(h).start()
                cp_v(h).start()
            cp_wo.start()
            cp_win2.start()
            cp_win1.start()
            for c_ in cp_wout:
                c_.start()

            cp_c.wait()
            c = c_v[...].astype(F32)
            sc = _rows8(c * jax.nn.sigmoid(c)).astype(BF16)
            cp_mod.wait()
            mod = jnp.dot(sc, wmod_v[...], preferred_element_type=F32)
            sa, ca, ga, sb, cb, gb = (mod[:, i * D:(i + 1) * D] for i in range(6))
            vec_s[GA] = ga
            vec_s[SB] = sb
            vec_s[CB] = cb
            vec_s[GB] = gb

            cp_x.wait()
            x = _rows8(x_v[0].astype(F32))
            vec_s[X] = x
            h1 = _layernorm(x) * (1.0 + ca) + sa
            cp_wq.wait()
            q = jnp.dot(h1.astype(BF16), wq_v[...], preferred_element_type=F32)
            row = lax.broadcasted_iota(jnp.int32, (8, DH), 0)
            for j in range(HKV):
                qa = q[:, (2 * j) * DH:(2 * j + 1) * DH]
                qb = q[:, (2 * j + 1) * DH:(2 * j + 2) * DH]
                q_s[j] = jnp.where(row == 0, qa, qb)

            def head(j, carry):
                cp_k(j).wait()
                qj = q_s[j].astype(BF16)
                s = lax.dot_general(qj, k_v[j], _NT, preferred_element_type=F32)
                s = s * (DH ** -0.5)
                m = jnp.max(s, axis=-1, keepdims=True)
                p = jnp.exp(s - m)
                l = jnp.sum(p, axis=-1, keepdims=True)
                cp_v(j).wait()
                o = jnp.dot(p.astype(BF16), v_v[j], preferred_element_type=F32)
                o = o / l
                o_s[2 * j] = _rows8(o[0:1, :])
                o_s[2 * j + 1] = _rows8(o[1:2, :])
                return carry

            lax.fori_loop(0, HKV, head, 0)

            cp_wsp.wait()
            cp_bsp.wait()
            wsp = wsp_v[...].astype(F32)
            bsp = bsp_v[...].astype(F32).reshape(1, 1)

            o_all = jnp.concatenate([o_s[i] for i in range(HQ)], axis=1)
            o_all = o_all.astype(BF16)
            cp_wo.wait()
            y = lax.dot_general(o_all, wot_v[...], _NT, preferred_element_type=F32)
            x1 = vec_s[X] + vec_s[GA] * y
            vec_s[X1] = x1

            h2 = (_layernorm(x1) * (1.0 + vec_s[CB]) + vec_s[SB]).astype(BF16)
            cp_win2.wait()
            z2 = jnp.dot(h2, win_v[:, FH:], preferred_element_type=F32)
            g = wsp * _layernorm(jax.nn.gelu(z2, approximate=True)) + bsp
            cp_win1.wait()
            z1 = jnp.dot(h2, win_v[:, :FH], preferred_element_type=F32)
            u = (jax.nn.gelu(z1, approximate=True) * g).astype(BF16)

            for i, (r0, r1) in enumerate(_OUT_CHUNKS):
                cp_wout[i].wait()
                y2 = lax.dot_general(u, woutt_v[r0:r1, :], _NT,
                                     preferred_element_type=F32)
                res = vec_s[X1, :, r0:r1] + vec_s[GB, :, r0:r1] * y2
                o_ref[0, :, r0:r1] = res[0:1, :].astype(o_ref.dtype)

        pl.run_scoped(body, pltpu.SemaphoreType.DMA((n_sems,)))

    return kernel


@jax.jit
def pallas_adaLN_cond__sliding_block_cached__mixer_gmlp__decode_kernel(
    A_x: jax.Array,
    A_k_cache: jax.Array,
    A_v_cache: jax.Array,
    A_wq: jax.Array,
    A_wo: jax.Array,
    B_x: jax.Array,
    B_w_in: jax.Array,
    B_w_sp: jax.Array,
    B_b_sp: jax.Array,
    B_w_out: jax.Array,
    c: jax.Array,
    w_mod: jax.Array,
):
    del B_x
    assert A_x.shape == (1, 1, D) and c.shape == (1, D)
    assert A_k_cache.shape[:2] == (1, HKV) and A_k_cache.shape[3] == DH
    assert A_v_cache.shape == A_k_cache.shape
    assert A_wq.shape == (D, HQ * DH) and A_wo.shape == (HQ * DH, D)
    assert B_w_in.shape == (D, 2 * FH) and B_w_out.shape == (FH, D)
    assert B_w_sp.shape == (1, 1) and B_b_sp.shape == (1,)
    assert w_mod.shape == (D, 6 * D)
    sk = A_k_cache.shape[2]
    w = min(4096, max(256, sk // 4))
    assert w % 128 == 0 and (sk - w) % 16 == 0

    dt = A_x.dtype
    hbm = pl.BlockSpec(memory_space=pltpu.HBM)
    return pl.pallas_call(
        _make_kernel(sk, w),
        out_shape=jax.ShapeDtypeStruct((1, 1, D), dt),
        in_specs=[hbm] * 11,
        out_specs=pl.BlockSpec(memory_space=pltpu.VMEM),
        scratch_shapes=[
            pltpu.VMEM(A_x.shape, dt),
            pltpu.VMEM(c.shape, c.dtype),
            pltpu.VMEM(B_w_sp.shape, B_w_sp.dtype),
            pltpu.VMEM(B_b_sp.shape, B_b_sp.dtype),
            pltpu.VMEM(w_mod.shape, w_mod.dtype),
            pltpu.VMEM(A_wq.shape, A_wq.dtype),
            pltpu.VMEM((HKV, w, DH), A_k_cache.dtype),
            pltpu.VMEM((HKV, w, DH), A_v_cache.dtype),
            pltpu.VMEM((D, HQ * DH), A_wo.dtype),
            pltpu.VMEM(B_w_in.shape, B_w_in.dtype),
            pltpu.VMEM((D, FH), B_w_out.dtype),
            pltpu.VMEM((HKV, 8, DH), F32),
            pltpu.VMEM((HQ, 8, DH), F32),
            pltpu.VMEM((6, 8, D), F32),
        ],
        compiler_params=pltpu.CompilerParams(vmem_limit_bytes=64 * 1024 * 1024),
    )(A_x, A_k_cache, A_v_cache, A_wq, A_wo.T, B_w_in, B_w_sp, B_b_sp,
      B_w_out.T, c, w_mod)
```

```python
import jax
import jax.numpy as jnp
from jax import lax
import jax.experimental.pallas as pl
import jax.experimental.pallas.tpu as pltpu

D = 448
HQ, HKV, DH = 16, 8, 256
FH = 896
EPS = 1e-5
BF16 = jnp.bfloat16
F32 = jnp.float32

_NT = (((1,), (1,)), ((), ()))

_OUT_CHUNKS = ((0, 128), (128, 256), (256, 384), (384, 448))


def _layernorm(x):
    m = jnp.mean(x, axis=-1, keepdims=True)
    xc = x - m
    v = jnp.mean(xc * xc, axis=-1, keepdims=True)
    return xc * lax.rsqrt(v + EPS)


def _rows8(x):
    return jnp.broadcast_to(x, (8, x.shape[-1]))


def _make_kernel(sk, w):
    n_chunks = len(_OUT_CHUNKS)
    S_C, S_X, S_MOD, S_WQ, S_WSP, S_BSP = range(6)
    S_K, S_V = 6, 6 + HKV
    S_WO, S_WIN2, S_WIN1, S_WOUT = range(6 + 2 * HKV, 10 + 2 * HKV)
    n_sems = S_WOUT + n_chunks
    X, GA, SB, CB, GB, X1 = range(6)

    def kernel(x_hbm, k_hbm, v_hbm, wq_hbm, wot_hbm, win_hbm, wsp_hbm, bsp_hbm,
               woutt_hbm, c_hbm, wmod_hbm,
               o_ref,
               x_v, c_v, wsp_v, bsp_v, wmod_v, wq_v, k_v, v_v, wot_v, win_v,
               woutt_v, q_s, o_s, vec_s):

        def body(sems):
            cp = pltpu.make_async_copy
            cp_c = cp(c_hbm, c_v, sems.at[S_C])
            cp_x = cp(x_hbm, x_v, sems.at[S_X])
            cp_mod = cp(wmod_hbm, wmod_v, sems.at[S_MOD])
            cp_wq = cp(wq_hbm, wq_v, sems.at[S_WQ])
            cp_wsp = cp(wsp_hbm, wsp_v, sems.at[S_WSP])
            cp_bsp = cp(bsp_hbm, bsp_v, sems.at[S_BSP])

            def cp_k(h):
                return cp(k_hbm.at[0, h, pl.ds(sk - w, w), :], k_v.at[h],
                          sems.at[S_K + h])

            def cp_v(h):
                return cp(v_hbm.at[0, h, pl.ds(sk - w, w), :], v_v.at[h],
                          sems.at[S_V + h])

            cp_wo = cp(wot_hbm, wot_v, sems.at[S_WO])
            cp_win2 = cp(win_hbm.at[:, pl.ds(FH, FH)], win_v.at[:, pl.ds(FH, FH)],
                         sems.at[S_WIN2])
            cp_win1 = cp(win_hbm.at[:, pl.ds(0, FH)], win_v.at[:, pl.ds(0, FH)],
                         sems.at[S_WIN1])
            cp_wout = [
                cp(woutt_hbm.at[pl.ds(r0, r1 - r0), :],
                   woutt_v.at[pl.ds(r0, r1 - r0), :], sems.at[S_WOUT + i])
                for i, (r0, r1) in enumerate(_OUT_CHUNKS)
            ]

            cp_c.start()
            cp_x.start()
            cp_mod.start()
            cp_wq.start()
            cp_wsp.start()
            cp_bsp.start()
            for h in range(HKV):
                cp_k(h).start()
                cp_v(h).start()
            cp_wo.start()
            cp_win2.start()
            cp_win1.start()
            for c_ in cp_wout:
                c_.start()

            cp_c.wait()
            c = c_v[...].astype(F32)
            sc = _rows8(c * jax.nn.sigmoid(c)).astype(BF16)
            cp_mod.wait()
            mod = jnp.dot(sc, wmod_v[...], preferred_element_type=F32)
            sa, ca, ga, sb, cb, gb = (mod[:, i * D:(i + 1) * D] for i in range(6))
            vec_s[GA] = ga
            vec_s[SB] = sb
            vec_s[CB] = cb
            vec_s[GB] = gb

            cp_x.wait()
            x = _rows8(x_v[0].astype(F32))
            vec_s[X] = x
            h1 = _layernorm(x) * (1.0 + ca) + sa
            cp_wq.wait()
            q = jnp.dot(h1.astype(BF16), wq_v[...], preferred_element_type=F32)
            row = lax.broadcasted_iota(jnp.int32, (8, DH), 0)
            for j in range(HKV):
                qa = q[:, (2 * j) * DH:(2 * j + 1) * DH]
                qb = q[:, (2 * j + 1) * DH:(2 * j + 2) * DH]
                q_s[j] = jnp.where(row == 0, qa, qb)

            def head(j, carry):
                cp_k(j).wait()
                qj = q_s[j].astype(BF16)
                s = lax.dot_general(qj, k_v[j], _NT, preferred_element_type=F32)
                s = s * (DH ** -0.5)
                m = jnp.max(s, axis=-1, keepdims=True)
                p = jnp.exp(s - m)
                l = jnp.sum(p, axis=-1, keepdims=True)
                cp_v(j).wait()
                o = jnp.dot(p.astype(BF16), v_v[j], preferred_element_type=F32)
                o = o / l
                o_s[2 * j] = _rows8(o[0:1, :])
                o_s[2 * j + 1] = _rows8(o[1:2, :])
                return carry

            lax.fori_loop(0, HKV, head, 0)

            cp_wsp.wait()
            cp_bsp.wait()
            wsp = wsp_v[...].astype(F32)
            bsp = bsp_v[...].astype(F32).reshape(1, 1)

            o_all = jnp.concatenate([o_s[i] for i in range(HQ)], axis=1)
            o_all = o_all.astype(BF16)
            cp_wo.wait()
            y = lax.dot_general(o_all, wot_v[...], _NT, preferred_element_type=F32)
            x1 = vec_s[X] + vec_s[GA] * y
            vec_s[X1] = x1

            h2 = (_layernorm(x1) * (1.0 + vec_s[CB]) + vec_s[SB]).astype(BF16)
            cp_win2.wait()
            z2 = jnp.dot(h2, win_v[:, FH:], preferred_element_type=F32)
            g = wsp * _layernorm(jax.nn.gelu(z2, approximate=True)) + bsp
            cp_win1.wait()
            z1 = jnp.dot(h2, win_v[:, :FH], preferred_element_type=F32)
            u = (jax.nn.gelu(z1, approximate=True) * g).astype(BF16)

            y2 = []
            for i, (r0, r1) in enumerate(_OUT_CHUNKS):
                cp_wout[i].wait()
                y2.append(lax.dot_general(u, woutt_v[r0:r1, :], _NT,
                                          preferred_element_type=F32))
            for (r0, r1), y2_blk in zip(_OUT_CHUNKS, y2):
                res = vec_s[X1, :, r0:r1] + vec_s[GB, :, r0:r1] * y2_blk
                o_ref[0, :, r0:r1] = res[0:1, :].astype(o_ref.dtype)

        pl.run_scoped(body, pltpu.SemaphoreType.DMA((n_sems,)))

    return kernel


@jax.jit
def pallas_adaLN_cond__sliding_block_cached__mixer_gmlp__decode_kernel(
    A_x: jax.Array,
    A_k_cache: jax.Array,
    A_v_cache: jax.Array,
    A_wq: jax.Array,
    A_wo: jax.Array,
    B_x: jax.Array,
    B_w_in: jax.Array,
    B_w_sp: jax.Array,
    B_b_sp: jax.Array,
    B_w_out: jax.Array,
    c: jax.Array,
    w_mod: jax.Array,
):
    del B_x
    assert A_x.shape == (1, 1, D) and c.shape == (1, D)
    assert A_k_cache.shape[:2] == (1, HKV) and A_k_cache.shape[3] == DH
    assert A_v_cache.shape == A_k_cache.shape
    assert A_wq.shape == (D, HQ * DH) and A_wo.shape == (HQ * DH, D)
    assert B_w_in.shape == (D, 2 * FH) and B_w_out.shape == (FH, D)
    assert B_w_sp.shape == (1, 1) and B_b_sp.shape == (1,)
    assert w_mod.shape == (D, 6 * D)
    sk = A_k_cache.shape[2]
    w = min(4096, max(256, sk // 4))
    assert w % 128 == 0 and (sk - w) % 16 == 0

    dt = A_x.dtype
    hbm = pl.BlockSpec(memory_space=pltpu.HBM)
    return pl.pallas_call(
        _make_kernel(sk, w),
        out_shape=jax.ShapeDtypeStruct((1, 1, D), dt),
        in_specs=[hbm] * 11,
        out_specs=pl.BlockSpec(memory_space=pltpu.VMEM),
        scratch_shapes=[
            pltpu.VMEM(A_x.shape, dt),
            pltpu.VMEM(c.shape, c.dtype),
            pltpu.VMEM(B_w_sp.shape, B_w_sp.dtype),
            pltpu.VMEM(B_b_sp.shape, B_b_sp.dtype),
            pltpu.VMEM(w_mod.shape, w_mod.dtype),
            pltpu.VMEM(A_wq.shape, A_wq.dtype),
            pltpu.VMEM((HKV, w, DH), A_k_cache.dtype),
            pltpu.VMEM((HKV, w, DH), A_v_cache.dtype),
            pltpu.VMEM((D, HQ * DH), A_wo.dtype),
            pltpu.VMEM(B_w_in.shape, B_w_in.dtype),
            pltpu.VMEM((D, FH), B_w_out.dtype),
            pltpu.VMEM((HKV, 8, DH), F32),
            pltpu.VMEM((HQ, 8, DH), F32),
            pltpu.VMEM((6, 8, D), F32),
        ],
        compiler_params=pltpu.CompilerParams(vmem_limit_bytes=64 * 1024 * 1024),
    )(A_x, A_k_cache, A_v_cache, A_wq, A_wo.T, B_w_in, B_w_sp, B_b_sp,
      B_w_out.T, c, w_mod)
```

```python
import jax
import jax.numpy as jnp
from jax import lax
import jax.experimental.pallas as pl
import jax.experimental.pallas.tpu as pltpu

D = 448
HQ, HKV, DH = 16, 8, 256
FH = 896
EPS = 1e-5
BF16 = jnp.bfloat16
F32 = jnp.float32

_NT = (((1,), (1,)), ((), ()))

_OUT_CHUNKS = ((0, 128), (128, 256), (256, 384), (384, 448))


def _layernorm(x):
    m = jnp.mean(x, axis=-1, keepdims=True)
    xc = x - m
    v = jnp.mean(xc * xc, axis=-1, keepdims=True)
    return xc * lax.rsqrt(v + EPS)


def _rows8(x):
    return jnp.broadcast_to(x, (8, x.shape[-1]))


def _make_kernel(sk, w):
    n_chunks = len(_OUT_CHUNKS)
    S_C, S_X, S_MOD, S_WQ, S_WSP, S_BSP = range(6)
    S_K, S_V = 6, 6 + HKV
    S_WO, S_WIN2, S_WIN1, S_WOUT = range(6 + 2 * HKV, 10 + 2 * HKV)
    n_sems = S_WOUT + n_chunks
    X, GA, SB, CB, GB, X1 = range(6)

    def kernel(x_hbm, k_hbm, v_hbm, wq_hbm, wot_hbm, win_hbm, wsp_hbm, bsp_hbm,
               woutt_hbm, c_hbm, wmod_hbm,
               o_ref,
               x_v, c_v, wsp_v, bsp_v, wmod_v, wq_v, k_v, v_v, wot_v, win2_v,
               win1_v, *rest):
        woutt_v, (q_s, o_s, vec_s) = rest[:n_chunks], rest[n_chunks:]

        def body(sems):
            cp = pltpu.make_async_copy
            cp_c = cp(c_hbm, c_v, sems.at[S_C])
            cp_x = cp(x_hbm, x_v, sems.at[S_X])
            cp_mod = cp(wmod_hbm, wmod_v, sems.at[S_MOD])
            cp_wq = cp(wq_hbm, wq_v, sems.at[S_WQ])
            cp_wsp = cp(wsp_hbm, wsp_v, sems.at[S_WSP])
            cp_bsp = cp(bsp_hbm, bsp_v, sems.at[S_BSP])

            def cp_k(h):
                return cp(k_hbm.at[0, h, pl.ds(sk - w, w), :], k_v.at[h],
                          sems.at[S_K + h])

            def cp_v(h):
                return cp(v_hbm.at[0, h, pl.ds(sk - w, w), :], v_v.at[h],
                          sems.at[S_V + h])

            cp_wo = cp(wot_hbm, wot_v, sems.at[S_WO])
            cp_win2 = cp(win_hbm.at[:, pl.ds(FH, FH)], win2_v, sems.at[S_WIN2])
            cp_win1 = cp(win_hbm.at[:, pl.ds(0, FH)], win1_v, sems.at[S_WIN1])
            cp_wout = [
                cp(woutt_hbm.at[pl.ds(r0, r1 - r0), :], woutt_v[i],
                   sems.at[S_WOUT + i])
                for i, (r0, r1) in enumerate(_OUT_CHUNKS)
            ]

            cp_c.start()
            cp_x.start()
            cp_mod.start()
            cp_wq.start()
            cp_wsp.start()
            cp_bsp.start()
            for h in range(HKV):
                cp_k(h).start()
                cp_v(h).start()
            cp_wo.start()
            cp_win2.start()
            cp_win1.start()
            for c_ in cp_wout:
                c_.start()

            cp_c.wait()
            c = c_v[...].astype(F32)
            sc = _rows8(c * jax.nn.sigmoid(c)).astype(BF16)
            cp_mod.wait()
            mod = jnp.dot(sc, wmod_v[...], preferred_element_type=F32)
            sa, ca, ga, sb, cb, gb = (mod[:, i * D:(i + 1) * D] for i in range(6))
            vec_s[GA] = ga
            vec_s[SB] = sb
            vec_s[CB] = cb
            vec_s[GB] = gb

            cp_x.wait()
            x = _rows8(x_v[0].astype(F32))
            vec_s[X] = x
            h1 = _layernorm(x) * (1.0 + ca) + sa
            cp_wq.wait()
            q = jnp.dot(h1.astype(BF16), wq_v[...], preferred_element_type=F32)
            row = lax.broadcasted_iota(jnp.int32, (8, DH), 0)
            for j in range(HKV):
                qa = q[:, (2 * j) * DH:(2 * j + 1) * DH]
                qb = q[:, (2 * j + 1) * DH:(2 * j + 2) * DH]
                q_s[j] = jnp.where(row == 0, qa, qb)

            def head(j, carry):
                cp_k(j).wait()
                qj = q_s[j].astype(BF16)
                s = lax.dot_general(qj, k_v[j], _NT, preferred_element_type=F32)
                s = s * (DH ** -0.5)
                m = jnp.max(s, axis=-1, keepdims=True)
                p = jnp.exp(s - m)
                l = jnp.sum(p, axis=-1, keepdims=True)
                cp_v(j).wait()
                o = jnp.dot(p.astype(BF16), v_v[j], preferred_element_type=F32)
                o = o / l
                o_s[2 * j] = _rows8(o[0:1, :])
                o_s[2 * j + 1] = _rows8(o[1:2, :])
                return carry

            lax.fori_loop(0, HKV, head, 0)

            cp_wsp.wait()
            cp_bsp.wait()
            wsp = wsp_v[...].astype(F32)
            bsp = bsp_v[...].astype(F32).reshape(1, 1)

            o_all = jnp.concatenate([o_s[i] for i in range(HQ)], axis=1)
            o_all = o_all.astype(BF16)
            cp_wo.wait()
            y = lax.dot_general(o_all, wot_v[...], _NT, preferred_element_type=F32)
            x1 = vec_s[X] + vec_s[GA] * y
            vec_s[X1] = x1

            h2 = (_layernorm(x1) * (1.0 + vec_s[CB]) + vec_s[SB]).astype(BF16)
            cp_win2.wait()
            z2 = jnp.dot(h2, win2_v[...], preferred_element_type=F32)
            g = wsp * _layernorm(jax.nn.gelu(z2, approximate=True)) + bsp
            cp_win1.wait()
            z1 = jnp.dot(h2, win1_v[...], preferred_element_type=F32)
            u = (jax.nn.gelu(z1, approximate=True) * g).astype(BF16)

            y2 = []
            for i, (r0, r1) in enumerate(_OUT_CHUNKS):
                cp_wout[i].wait()
                y2.append(lax.dot_general(u, woutt_v[i][...], _NT,
                                          preferred_element_type=F32))
            for (r0, r1), y2_blk in zip(_OUT_CHUNKS, y2):
                res = vec_s[X1, :, r0:r1] + vec_s[GB, :, r0:r1] * y2_blk
                o_ref[0, :, r0:r1] = res[0:1, :].astype(o_ref.dtype)

        pl.run_scoped(body, pltpu.SemaphoreType.DMA((n_sems,)))

    return kernel


@jax.jit
def pallas_adaLN_cond__sliding_block_cached__mixer_gmlp__decode_kernel(
    A_x: jax.Array,
    A_k_cache: jax.Array,
    A_v_cache: jax.Array,
    A_wq: jax.Array,
    A_wo: jax.Array,
    B_x: jax.Array,
    B_w_in: jax.Array,
    B_w_sp: jax.Array,
    B_b_sp: jax.Array,
    B_w_out: jax.Array,
    c: jax.Array,
    w_mod: jax.Array,
):
    del B_x
    assert A_x.shape == (1, 1, D) and c.shape == (1, D)
    assert A_k_cache.shape[:2] == (1, HKV) and A_k_cache.shape[3] == DH
    assert A_v_cache.shape == A_k_cache.shape
    assert A_wq.shape == (D, HQ * DH) and A_wo.shape == (HQ * DH, D)
    assert B_w_in.shape == (D, 2 * FH) and B_w_out.shape == (FH, D)
    assert B_w_sp.shape == (1, 1) and B_b_sp.shape == (1,)
    assert w_mod.shape == (D, 6 * D)
    sk = A_k_cache.shape[2]
    w = min(4096, max(256, sk // 4))
    assert w % 128 == 0 and (sk - w) % 16 == 0

    dt = A_x.dtype
    hbm = pl.BlockSpec(memory_space=pltpu.HBM)
    return pl.pallas_call(
        _make_kernel(sk, w),
        out_shape=jax.ShapeDtypeStruct((1, 1, D), dt),
        in_specs=[hbm] * 11,
        out_specs=pl.BlockSpec(memory_space=pltpu.VMEM),
        scratch_shapes=[
            pltpu.VMEM(A_x.shape, dt),
            pltpu.VMEM(c.shape, c.dtype),
            pltpu.VMEM(B_w_sp.shape, B_w_sp.dtype),
            pltpu.VMEM(B_b_sp.shape, B_b_sp.dtype),
            pltpu.VMEM(w_mod.shape, w_mod.dtype),
            pltpu.VMEM(A_wq.shape, A_wq.dtype),
            pltpu.VMEM((HKV, w, DH), A_k_cache.dtype),
            pltpu.VMEM((HKV, w, DH), A_v_cache.dtype),
            pltpu.VMEM((D, HQ * DH), A_wo.dtype),
            pltpu.VMEM((D, FH), B_w_in.dtype),
            pltpu.VMEM((D, FH), B_w_in.dtype),
        ] + [
            pltpu.VMEM((r1 - r0, FH), B_w_out.dtype)
            for r0, r1 in _OUT_CHUNKS
        ] + [
            pltpu.VMEM((HKV, 8, DH), F32),
            pltpu.VMEM((HQ, 8, DH), F32),
            pltpu.VMEM((6, 8, D), F32),
        ],
        compiler_params=pltpu.CompilerParams(vmem_limit_bytes=64 * 1024 * 1024),
    )(A_x, A_k_cache, A_v_cache, A_wq, A_wo.T, B_w_in, B_w_sp, B_b_sp,
      B_w_out.T, c, w_mod)
```
